```python
import os as _os
_os.environ.setdefault("JAX_PLATFORMS", "cpu")
import jax
import jax.numpy as jnp

def _softmax(x, axis=-1):
    return jax.nn.softmax(x, axis=axis)
def _gelu(x):
    return jax.nn.gelu(x, approximate=True)
def _silu(x):
    return jax.nn.silu(x)
def _sigmoid(x):
    return jax.nn.sigmoid(x)
def _layernorm(x, axis=-1, eps=1e-5):
    m = jnp.mean(x, axis=axis, keepdims=True)
    v = jnp.var(x, axis=axis, keepdims=True)
    return (x - m) / jnp.sqrt(v + eps)
def _scatter_add(tgt, idx, src, axis=0):
    return tgt.at[idx].add(src)
def _segment_sum(src, seg, n):
    return jax.ops.segment_sum(src, seg, n)
class _Rng:
    def __init__(self, key):
        self._k = key
    def _next(self):
        self._k, sub = jax.random.split(self._k)
        return sub
    def normal(self, shape):
        return jax.random.normal(self._next(), shape, dtype=jnp.bfloat16)
    def randint(self, lo, hi, shape):
        return jax.random.randint(self._next(), shape, lo, hi, dtype=jnp.int32)
    def uniform(self, shape, lo=0.0, hi=1.0):
        return jax.random.uniform(self._next(), shape, jnp.bfloat16, lo, hi)
    def permutation(self, n):
        return jax.random.permutation(self._next(), n)


kernel_name = 'standalone__linear_kernel_hedgehog__prompt'

def setup_inputs():
    _rng = _Rng(jax.random.key(int.from_bytes(__import__("os").urandom(4), "little")))
    _w = (lambda a: (lambda t: t.astype(jnp.bfloat16) if jnp.issubdtype(t.dtype, jnp.floating) else t)(jnp.asarray(a)))
    B, S, D, H = 1, 2048, 1024, 32
    Dh = D // H
    return {
        "x": _w((lambda *s: _rng.normal(s) * 0.4)(B, S, D)),
        "wqkv": _w((lambda *s: _rng.normal(s) * 0.4)(D, 3 * D)),
        "w_phi": _w((lambda *s: _rng.normal(s) * 0.4)(H, Dh, Dh) * (Dh ** -0.5)),
        "wo": _w((lambda *s: _rng.normal(s) * 0.05)(D, D)),
    }

def reference(x, wqkv, w_phi, wo):
    B, S, D = x.shape
    H = 32; Dh = D // H
    qkv = (lambda x, *d: x.transpose(*d))((x @ wqkv).reshape(B, S, 3, H, Dh), 2, 0, 3, 1, 4)
    q, k, v = qkv[0], qkv[1], qkv[2]
    pq = jnp.einsum("bhsd,hdf->bhsf", q, w_phi)
    pk = jnp.einsum("bhsd,hdf->bhsf", k, w_phi)
    phi_q = jnp.concatenate([_softmax(pq, axis=-1), _softmax(-pq, axis=-1)], axis=-1)
    phi_k = jnp.concatenate([_softmax(pk, axis=-1), _softmax(-pk, axis=-1)], axis=-1)
    kv = jnp.einsum("bhsf,bhsd->bhfd", phi_k, v)
    z  = jnp.einsum("bhsf->bhf", phi_k)
    num = jnp.einsum("bhqf,bhfd->bhqd", phi_q, kv)
    den = jnp.einsum("bhqf,bhf->bhq", phi_q, z)[..., None] + 1e-6
    o = num / den
    return (lambda x, *d: x.transpose(*d))(o, 0, 2, 1, 3).reshape(B, S, D) @ wo
```

```python
import functools
import numpy as np
import jax
import jax.numpy as jnp
from jax import lax
import jax.experimental.pallas as pl
import jax.experimental.pallas.tpu as pltpu

f32 = jnp.float32
bf16 = jnp.bfloat16
LOG2E = 1.4426950408889634
H = 32
DH = 32


def _nt(a, b):
    return lax.dot_general(a, b, (((1,), (1,)), ((), ())), preferred_element_type=f32)


def _nn(a, b):
    return jnp.dot(a, b, preferred_element_type=f32)


def _dual_softmax(p):
    R, Tn = p.shape
    p3 = p.reshape(R // DH, DH, Tn)
    mx = jnp.max(p3, axis=1, keepdims=True)
    mn = jnp.min(p3, axis=1, keepdims=True)
    ep = jnp.exp2(p3 - mx)
    en = jnp.exp2(mn - p3)
    sp = jnp.sum(ep, axis=1, keepdims=True)
    sn = jnp.sum(en, axis=1, keepdims=True)
    pp = ep * (1.0 / sp)
    pn = en * (1.0 / sn)
    return pp.reshape(R, Tn), pn.reshape(R, Tn)


def make_kernel(S, D, T):
    NB = S // T
    NP = H // 2

    def kernel(x_hbm, wqkv_hbm, wphi_hbm, wo_hbm, o_hbm,
               xs, wraw, wphi, wkT, wvT, wqT, wo, kv, zacc, kvbd, zb, ostage,
               xsem, wsem, osem):
        def x_copy(i):
            return pltpu.make_async_copy(x_hbm.at[pl.ds(i * T, T)], xs.at[pl.ds(i * T, T)], xsem.at[i])

        def w_copy(j):
            return pltpu.make_async_copy(wqkv_hbm.at[:, pl.ds(j * D, D)], wraw.at[j], wsem.at[j])

        phi_copy = pltpu.make_async_copy(wphi_hbm, wphi, wsem.at[3])
        wo_copy = pltpu.make_async_copy(wo_hbm, wo, wsem.at[4])

        phi_copy.start()
        w_copy(1).start()
        w_copy(2).start()
        for i in range(NB):
            x_copy(i).start()
        w_copy(0).start()
        wo_copy.start()

        phi_copy.wait()

        rows = lax.broadcasted_iota(jnp.int32, (128, 128), 0) // DH
        cols = lax.broadcasted_iota(jnp.int32, (128, 128), 1) // DH
        bd_mask = rows == cols

        def wprep(j, dst):
            for g in range(H // 4):
                w4 = wphi[4 * g:4 * g + 4].reshape(128, DH)
                w4 = jnp.concatenate([w4] * 4, axis=1)
                bg = jnp.where(bd_mask, w4, jnp.zeros_like(w4)).astype(f32)
                ag = bg.T.astype(bf16)
                wt = _nt(ag, wraw[j, :, 128 * g:128 * (g + 1)])
                dst[128 * g:128 * (g + 1), :] = (wt * LOG2E).astype(bf16)

        w_copy(1).wait()
        wprep(1, wkT)
        w_copy(2).wait()
        for g in range(D // 128):
            wvT[128 * g:128 * (g + 1), :] = wraw[2, :, 128 * g:128 * (g + 1)].astype(f32).T.astype(bf16)

        kv[...] = jnp.zeros_like(kv)
        zacc[...] = jnp.zeros_like(zacc)

        def kbody(i, c):
            x_copy(i).wait()
            s0 = pl.multiple_of(i * T, T)
            xb = xs[pl.ds(s0, T), :]
            pk = _nt(wkT[...], xb)
            vT = _nt(wvT[...], xb).astype(bf16)
            pp, pn = _dual_softmax(pk)
            zp = pp[:, 0:128]
            zn = pn[:, 0:128]
            for j in range(1, T // 128):
                zp = zp + pp[:, j * 128:(j + 1) * 128]
                zn = zn + pn[:, j * 128:(j + 1) * 128]
            zacc[0] += zp
            zacc[1] += zn
            pp = pp.astype(bf16)
            pn = pn.astype(bf16)
            for p in range(NP):
                tile = jnp.concatenate([pp[64 * p:64 * p + 64], pn[64 * p:64 * p + 64]], axis=0)
                kv[p] += _nt(vT[64 * p:64 * p + 64], tile)
            return c

        lax.fori_loop(0, NB, kbody, 0)

        w_copy(0).wait()
        wprep(0, wqT)
        wo_copy.wait()

        r2 = lax.broadcasted_iota(jnp.int32, (64, 128), 0) // 32
        c2 = (lax.broadcasted_iota(jnp.int32, (64, 128), 1) // 32) % 2
        m2 = r2 == c2
        for p in range(NP):
            kvbd[p] = jnp.where(m2, kv[p], 0.0).astype(bf16)
        for s in range(2):
            zs = jnp.sum(zacc[s], axis=1, keepdims=True)
            zb[s] = jnp.broadcast_to(zs, (D, 128))

        def o_copy(i, slot):
            return pltpu.make_async_copy(ostage.at[slot], o_hbm.at[pl.ds(pl.multiple_of(i * T, T), T)], osem.at[slot])

        def qbody(i, c):
            slot = i % 2
            s0 = pl.multiple_of(i * T, T)
            xb = xs[pl.ds(s0, T), :]
            pq = _nt(wqT[...], xb)
            pp, pn = _dual_softmax(pq)
            zbp = jnp.concatenate([zb[0]] * (T // 128), axis=1)
            zbn = jnp.concatenate([zb[1]] * (T // 128), axis=1)
            den = jnp.sum((pp * zbp + pn * zbn).reshape(H, DH, T), axis=1, keepdims=True)
            rden = 1.0 / (den + 1e-6)
            pp = pp.astype(bf16)
            pn = pn.astype(bf16)
            nums = []
            for p in range(NP):
                tile = jnp.concatenate([pp[64 * p:64 * p + 64], pn[64 * p:64 * p + 64]], axis=0)
                nums.append(_nn(kvbd[p], tile))
            numT = jnp.concatenate(nums, axis=0)
            oT = (numT.reshape(H, DH, T) * rden).reshape(D, T)
            o = oT.T.astype(bf16)
            out = _nn(o, wo[...]).astype(bf16)

            @pl.when(i >= 2)
            def _():
                o_copy(i - 2, slot).wait()

            ostage[slot] = out
            o_copy(i, slot).start()
            return c

        lax.fori_loop(0, NB, qbody, 0)
        for i in range(NB - 2, NB):
            o_copy(i, i % 2).wait()

    return kernel


@jax.jit
def pallas_standalone__linear_kernel_hedgehog__prompt_kernel(x, wqkv, w_phi, wo):
    B, S, D = x.shape
    T = 512
    x2 = x.reshape(S, D)
    out = pl.pallas_call(
        make_kernel(S, D, T),
        out_shape=jax.ShapeDtypeStruct((S, D), bf16),
        in_specs=[pl.BlockSpec(memory_space=pl.ANY)] * 4,
        out_specs=pl.BlockSpec(memory_space=pl.ANY),
        scratch_shapes=[
            pltpu.VMEM((S, D), bf16),
            pltpu.VMEM((3, D, D), bf16),
            pltpu.VMEM((H, DH, DH), bf16),
            pltpu.VMEM((D, D), bf16),
            pltpu.VMEM((D, D), bf16),
            pltpu.VMEM((D, D), bf16),
            pltpu.VMEM((D, D), bf16),
            pltpu.VMEM((H // 2, 64, 128), f32),
            pltpu.VMEM((2, D, 128), f32),
            pltpu.VMEM((H // 2, 64, 128), bf16),
            pltpu.VMEM((2, D, 128), f32),
            pltpu.VMEM((2, T, D), bf16),
            pltpu.SemaphoreType.DMA((S // T,)),
            pltpu.SemaphoreType.DMA((5,)),
            pltpu.SemaphoreType.DMA((2,)),
        ],
        compiler_params=pltpu.CompilerParams(vmem_limit_bytes=100 * 1024 * 1024),
    )(x2, wqkv, w_phi, wo)
    return out.reshape(B, S, D)
```

```python
import numpy as np
import jax
import jax.numpy as jnp
from jax import lax
import jax.experimental.pallas as pl
import jax.experimental.pallas.tpu as pltpu

f32 = jnp.float32
bf16 = jnp.bfloat16
u32 = jnp.uint32
LOG2E = 1.4426950408889634
H = 32
DH = 32


def _nt(a, b):
    return lax.dot_general(a, b, (((1,), (1,)), ((), ())), preferred_element_type=f32)


def _nn(a, b):
    return jnp.dot(a, b, preferred_element_type=f32)


def _pk(x):
    return pltpu.bitcast(x.astype(bf16), u32)


def _up(x):
    return pltpu.bitcast(x, bf16)


def _rcp(s):
    r = pltpu.reciprocal(s, approx=True)
    return r * (2.0 - s * r)


def _allred(x, op):
    x = op(x, pltpu.roll(x, 4, 1))
    return op(x, pltpu.roll(x, 2, 1))


def _dual_softmax(p):
    R, Tn = p.shape
    p4 = p.reshape(R // 64, 8, 8, Tn)
    mx = _allred(jnp.max(p4, axis=1), jnp.maximum)[:, None]
    mn = _allred(jnp.min(p4, axis=1), jnp.minimum)[:, None]
    ep = jnp.exp2(p4 - mx)
    en = jnp.exp2(mn - p4)
    sp = _allred(jnp.sum(ep, axis=1), jnp.add)[:, None]
    sn = _allred(jnp.sum(en, axis=1), jnp.add)[:, None]
    pp = ep * _rcp(sp)
    pn = en * _rcp(sn)
    return jnp.concatenate([pp.reshape(R, Tn), pn.reshape(R, Tn)], axis=0)


def _lhs_ops(a11, a12, a21, a22):
    return [(a11 + a22), (a21 + a22), a11, a22, (a11 + a12), (a21 - a11), (a12 - a22)]


def _rhs_ops(b11, b12, b21, b22):
    return [(b11 + b22), b11, (b12 - b22), (b21 - b11), b22, (b11 + b12), (b21 + b22)]


class _Fill:
    def __init__(self, thunks):
        self.t = list(thunks)

    def pop(self, n=1):
        for _ in range(min(n, len(self.t))):
            self.t.pop(0)()

    def drain(self):
        self.pop(len(self.t))


def make_kernel(S, D, T):
    NB = S // T
    NP = H // 2
    T2 = T // 2
    D2 = D // 2
    NG = 4

    def kernel(x_hbm, wqkv_hbm, wphi_hbm, wo_hbm, o_hbm,
               stg, xu, wphi, abd, vw, vv, uo, phq, phk, vts, kv, zacc, kvbd, vo, ostage,
               xsem, gsem, wsem, osem, fsem, rsem):
        def x_copy(i):
            return pltpu.make_async_copy(x_hbm.at[pl.ds(i * T, T)], stg.at[pl.ds(i * T, T)], xsem.at[i])

        WO = S

        def urow(u):
            return S + D + D * (u // NG) if isinstance(u, int) else pl.multiple_of(S + D + D * (u // NG), D)

        def ucol(u):
            return 256 * (u % NG) if isinstance(u, int) else pl.multiple_of(256 * (u % NG), 256)

        def u_copy(u):
            if isinstance(u, int):
                col = (D, 0, 2 * D)[u // NG] + 256 * (u % NG)
            else:
                blk = u // NG
                col = pl.multiple_of(jnp.where(blk == 0, D, jnp.where(blk == 1, 0, 2 * D)) + 256 * (u % NG), 256)
            return pltpu.make_async_copy(wqkv_hbm.at[:, pl.ds(col, 256)], stg.at[pl.ds(urow(u), D), pl.ds(ucol(u), 256)], gsem.at[u])

        phi_copy = pltpu.make_async_copy(wphi_hbm, wphi, wsem.at[0])
        wo_copy = pltpu.make_async_copy(wo_hbm, stg.at[pl.ds(WO, D)], wsem.at[1])

        phi_copy.start()
        pl.semaphore_signal(rsem, 1)
        pl.semaphore_wait(rsem, 1)
        u_copy(0).start()
        u_copy(8).start()
        x_copy(0).start()
        for g in range(1, NG):
            u_copy(g).start()
            u_copy(8 + g).start()
        for g in range(NG):
            u_copy(4 + g).start()
        x_copy(1).start()
        wo_copy.start()
        for i in range(2, NB):
            x_copy(i).start()

        def mo(v, m):
            return v if isinstance(v, int) else pl.multiple_of(v, m)

        def wprep(u):
            g = u % NG
            j = u // NG
            for hh in range(2):
                wt = _nt(_up(abd[pl.ds(mo(64 * (2 * g + hh), 64), 64), :]), stg[pl.ds(urow(u), D), pl.ds(mo(ucol(u) + 128 * hh, 128), 128)]) * LOG2E
                r0 = 64 * g + 32 * hh
                for c in range(D2 // 128):
                    lo = wt[:, 128 * c:128 * (c + 1)]
                    hi = wt[:, D2 + 128 * c:D2 + 128 * (c + 1)]
                    ops = _lhs_ops(lo[:64], hi[:64], lo[64:], hi[64:])
                    for n, op in enumerate(ops):
                        vw[pl.ds(mo((7 * j + n) * 256 + r0, 32), 32), 128 * c:128 * (c + 1)] = _pk(op)

        def vprep_thunks(g_src, g_dst):
            def one(hh, c):
                cs = pl.ds(mo(256 * g_src + 128 * hh, 128), 128)
                lo = stg[S + 3 * D + 128 * c:S + 3 * D + 128 * (c + 1), cs].T.astype(f32)
                hi = stg[S + 3 * D + D2 + 128 * c:S + 3 * D + D2 + 128 * (c + 1), cs].T.astype(f32)
                ops = _lhs_ops(lo[:64], hi[:64], lo[64:], hi[64:])
                r0 = 64 * g_dst + 32 * hh
                for n, op in enumerate(ops):
                    vv[pl.ds(mo(n * 320 + r0, 32), 32), 128 * c:128 * (c + 1)] = _pk(op)
            return [lambda hh=hh, c=c: one(hh, c) for hh in range(2) for c in range(D2 // 128)]

        def xsum_thunks(i, s0):
            def one(c):
                r = 16 * c
                x11 = stg[pl.ds(s0 + r, 16), 0:D2].astype(f32)
                x12 = stg[pl.ds(s0 + r, 16), D2:D].astype(f32)
                x21 = stg[pl.ds(s0 + T2 + r, 16), 0:D2].astype(f32)
                x22 = stg[pl.ds(s0 + T2 + r, 16), D2:D].astype(f32)
                for n, op in enumerate(_rhs_ops(x11, x21, x12, x22)):
                    xu[pl.ds(mo((7 * i + n) * 128 + 8 * c, 8), 8), :] = _pk(op)
            return [lambda c=c: one(c) for c in range(T2 // 16)]

        def wosum_thunks(s):
            def one(c):
                r0 = mo(128 * s + 16 * c, 16)
                b11 = stg[pl.ds(r0 + WO, 16), 0:D2].astype(f32)
                b12 = stg[pl.ds(r0 + WO, 16), D2:D].astype(f32)
                b21 = stg[pl.ds(r0 + WO + D2, 16), 0:D2].astype(f32)
                b22 = stg[pl.ds(r0 + WO + D2, 16), D2:D].astype(f32)
                q0 = 64 * s + 8 * c
                for n, op in enumerate(_rhs_ops(b11, b12, b21, b22)):
                    uo[pl.ds(mo(n * 256 + q0, 8), 8), :] = _pk(op)
            return [lambda c=c: one(c) for c in range(8)]

        def products(vref, i, r0, nr, emit, fill=None, per=1):
            def m(n):
                r = _nt(_up(vref(n, r0, nr // 2)), _up(xu[pl.ds(mo((7 * i + n) * 128, 128), 128), :]))
                if fill is not None:
                    fill.pop(per)
                return r
            m2 = m(1)
            m5 = m(4)
            m3 = m(2)
            t22 = m3 - m2
            m4 = m(3)
            emit(0, 1, m3 + m5)
            t11 = m4 - m5
            m1 = m(0)
            emit(1, 0, m2 + m4)
            t11 = t11 + m1
            t22 = t22 + m1
            m7 = m(6)
            m6 = m(5)
            emit(0, 0, t11 + m7)
            return lambda: emit(1, 1, t22 + m6)

        def half(r0):
            return r0 // 2 if isinstance(r0, int) else pl.multiple_of(r0 // 2, 64)

        vk_of = lambda n, r0, nr: vw[pl.ds(mo(n * 256 + r0, 64), nr), :]
        vq_of = lambda n, r0, nr: vw[pl.ds(mo((7 + n) * 256 + r0, 64), nr), :]
        vv_of = lambda n, r0, nr: vv[pl.ds(mo(n * 320 + r0, 64), nr), :]

        def k_emit(p0):
            def emit(fh, th, c):
                for sb in range(c.shape[0] // 64):
                    p = p0 + 2 * sb + fh
                    zs = None
                    for j in range(T2 // 128):
                        tl = _dual_softmax(c[64 * sb:64 * (sb + 1), 128 * j:128 * (j + 1)])
                        zs = tl if zs is None else zs + tl
                        t0 = T2 * th + 128 * j
                        phk[pl.ds(mo(64 * p, 64), 64), t0:t0 + 128] = _pk(tl)
                    zacc[p] += zs
            return emit

        def v_emit(p0):
            def emit(fh, th, c):
                for sb in range(c.shape[0] // 64):
                    vts[pl.ds(mo(32 * (p0 + 2 * sb + fh), 32), 32), T2 * th:T2 * (th + 1)] = _pk(c[64 * sb:64 * (sb + 1)])
            return emit

        def q_emit(i, p0):
            def emit(fh, th, c):
                for sb in range(c.shape[0] // 64):
                    p = p0 + 2 * sb + fh
                    for j in range(T2 // 128):
                        tl = _dual_softmax(c[64 * sb:64 * (sb + 1), 128 * j:128 * (j + 1)])
                        t0 = T2 * th + 128 * j
                        phq[pl.ds(mo(64 * (NP * i + p), 64), 64), t0:t0 + 128] = _pk(tl)
            return emit

        def kv_part(fill=None, per=1):
            for p in range(NP):
                kv[p] += _nt(_up(vts[32 * p:32 * (p + 1), :]), _up(phk[64 * p:64 * (p + 1), :]))
                if fill is not None:
                    fill.pop(per)

        def num_mm(i, jt):
            ps = [2 * jt, 2 * jt + 1, 8 + 2 * jt, 8 + 2 * jt + 1]
            return [_nn(_up(kvbd[40 * p:40 * (p + 1), :]), _up(phq[pl.ds(mo(64 * (NP * i + p), 64), 64), :])) for p in ps]

        def num_pair(res):
            rd = _rcp(res[64:80] + 1e-6).reshape(2, 1, 8, T)
            return (res[0:64].reshape(2, 4, 8, T) * rd).reshape(64, T)

        def ov_tile(nums):
            lo = jnp.concatenate([num_pair(nums[0]), num_pair(nums[1])], axis=0)
            hi = jnp.concatenate([num_pair(nums[2]), num_pair(nums[3])], axis=0)
            ops = _lhs_ops(lo[:, 0:T2], hi[:, 0:T2], lo[:, T2:T], hi[:, T2:T])
            return [_pk(op.astype(bf16).T) for op in ops]

        def vo_store(n, jt, val):
            vo[128 * n:128 * (n + 1), 128 * jt:128 * (jt + 1)] = val

        def o_copy(i):
            return pltpu.make_async_copy(ostage.at[i], o_hbm.at[pl.ds(pl.multiple_of(i * T, T), T)], osem.at[i])

        def oq_copy(i, th, nh):
            return pltpu.make_async_copy(
                ostage.at[i, pl.ds(th * T2, T2), pl.ds(nh * D2, D2)],
                o_hbm.at[pl.ds(i * T + th * T2, T2), pl.ds(nh * D2, D2)], fsem.at[2 * th + nh])

        def out_part(i, final, nxt=None):
            tiles = {}
            done = []
            stored = set()

            def flush():
                for n in done:
                    for jt in tiles:
                        if (n, jt) not in stored:
                            stored.add((n, jt))
                            vo_store(n, jt, tiles[jt][n])

            pend = []

            def step():
                if nxt is None:
                    return
                if pend:
                    jt, nums = pend.pop()
                    tiles[jt] = ov_tile(nums)
                jt = len(tiles)
                if jt < 4:
                    pend.append((jt, num_mm(nxt, jt)))

            def m(n):
                r = _nn(_up(vo[128 * n:128 * (n + 1), :]), _up(uo[256 * n:256 * (n + 1), :]))
                flush()
                done.append(n)
                step()
                return r
            step()
            m3 = m(2)
            m5 = m(4)
            ostage[i, 0:T2, D2:D] = (m3 + m5).astype(bf16)
            if final:
                oq_copy(i, 0, 1).start()
            m2 = m(1)
            t22 = m3 - m2
            m4 = m(3)
            ostage[i, T2:T, 0:D2] = (m2 + m4).astype(bf16)
            if final:
                oq_copy(i, 1, 0).start()
            t11 = m4 - m5
            m1 = m(0)
            t11 = t11 + m1
            t22 = t22 + m1
            m7 = m(6)
            ostage[i, 0:T2, 0:D2] = (t11 + m7).astype(bf16)
            if final:
                oq_copy(i, 0, 0).start()
            m6 = m(5)
            ostage[i, T2:T, D2:D] = (t22 + m6).astype(bf16)
            if final:
                oq_copy(i, 1, 1).start()
            flush()

        phi_copy.wait()
        r_s = lax.broadcasted_iota(jnp.int32, (128, DH), 0)
        c_s = lax.broadcasted_iota(jnp.int32, (128, DH), 1)
        sel = (((r_s % 64) // 2) == c_s).astype(f32).astype(bf16)
        r_m = lax.broadcasted_iota(jnp.int32, (128, 128), 0)
        c_m = lax.broadcasted_iota(jnp.int32, (128, 128), 1)
        hd_mask = (2 * (r_m // 64) + r_m % 2) == (c_m // DH)
        for gg in range(8):
            w4 = wphi[4 * gg:4 * gg + 4].reshape(128, DH)
            abd[64 * gg:64 * (gg + 1), :] = _pk(jnp.where(hd_mask, _nt(sel, w4), 0.0))
        for p in range(NP):
            kv[p] = jnp.zeros((64, 128), f32)
            zacc[p] = jnp.zeros((128, 128), f32)
        u_copy(0).wait()
        wprep(0)
        u_copy(8).wait()
        _Fill(vprep_thunks(0, 0)).drain()
        x_copy(0).wait()
        _Fill(xsum_thunks(0, 0)).drain()

        def pbody(g, c):
            u_copy(g + 1).wait()

            @pl.when(g < NG - 1)
            def _():
                u_copy(8 + g + 1).wait()

            r0 = pl.multiple_of(64 * g, 64)
            fill = _Fill(vprep_thunks(jnp.minimum(g + 1, NG - 1), g + 1))
            rest = products(vk_of, 0, r0, 128, k_emit(4 * g))
            wprep(g + 1)
            rest()
            rest = products(vv_of, 0, r0, 128, v_emit(4 * g), fill, 2)
            fill.drain()
            rest()
            return c

        lax.fori_loop(0, NG, pbody, 0)
        for g in range(1, NG):
            u_copy(4 + g).wait()
        wo_copy.wait()
        fill = _Fill(wosum_thunks(0))
        for g in range(1, NG):
            wprep(4 + g)
            fill.pop(3)

        def kbody(i, c):
            x_copy(i).wait()
            s0 = pl.multiple_of(i * T, T)
            fw = _Fill(wosum_thunks(i))
            kv_part(fw, 1)
            fx = _Fill(xsum_thunks(i, s0))
            rq = products(vq_of, i - 1, 0, D2, q_emit(i - 1, 0), fx, 3)
            fx.drain()
            rk = products(vk_of, i, 0, D2, k_emit(0), _Fill([rq]), 1)
            rv = products(vv_of, i, 0, D2, v_emit(0), _Fill([rk]), 1)
            rv()
            return c

        lax.fori_loop(1, NB, kbody, 0)

        kv_part()
        r0_ = products(vq_of, NB - 1, 0, 128, q_emit(NB - 1, 0))
        m2_ = (lax.broadcasted_iota(jnp.int32, (64, 128), 0) // 32) == (lax.broadcasted_iota(jnp.int32, (64, 128), 1) % 2)
        mz_ = (lax.broadcasted_iota(jnp.int32, (16, 128), 0) // 8) == (lax.broadcasted_iota(jnp.int32, (16, 128), 1) % 2)
        for p in range(NP):
            kvbd[40 * p:40 * p + 32, :] = _pk(jnp.where(m2_, kv[p], 0.0))
            zrow = jnp.sum(zacc[p].T, axis=0, keepdims=True)
            kvbd[40 * p + 32:40 * p + 40, :] = _pk(jnp.where(mz_, jnp.broadcast_to(zrow, (16, 128)), 0.0))

        def ov0(jt, nums):
            for n, val in enumerate(ov_tile(nums)):
                vo_store(n, jt, val)
        r0_()
        nm0 = num_mm(0, 0)
        nm1 = num_mm(0, 1)
        r1_ = products(vq_of, NB - 1, 64, 128, q_emit(NB - 1, 4))
        ov0(0, nm0)
        ov0(1, nm1)
        nm2 = num_mm(0, 2)
        nm3 = num_mm(0, 3)
        r2_ = products(vq_of, NB - 1, 128, 128, q_emit(NB - 1, 8), _Fill([r1_]), 1)
        ov0(2, nm2)
        ov0(3, nm3)
        r3_ = products(vq_of, NB - 1, 192, 128, q_emit(NB - 1, 12), _Fill([r2_]), 1)
        r3_()

        def qbody(i, c):
            out_part(i, False, i + 1)
            o_copy(i).start()
            return c

        lax.fori_loop(0, NB - 1, qbody, 0)

        out_part(NB - 1, True)
        for i in range(NB - 1):
            o_copy(i).wait()
        for th in range(2):
            for nh in range(2):
                oq_copy(NB - 1, th, nh).wait()

    return kernel


@jax.jit
def pallas_standalone__linear_kernel_hedgehog__prompt_kernel(x, wqkv, w_phi, wo):
    B, S, D = x.shape
    T = 512
    x2 = x.reshape(S, D)
    NB = S // T
    out = pl.pallas_call(
        make_kernel(S, D, T),
        out_shape=jax.ShapeDtypeStruct((S, D), bf16),
        in_specs=[pl.BlockSpec(memory_space=pl.ANY)] * 4,
        out_specs=pl.BlockSpec(memory_space=pl.ANY),
        scratch_shapes=[
            pltpu.VMEM((S + 4 * D, D), bf16),
            pltpu.VMEM((NB * 7 * T // 4, D // 2), u32),
            pltpu.VMEM((H, DH, DH), bf16),
            pltpu.VMEM((8 * 64, 128), u32),
            pltpu.VMEM((2 * 7 * D // 4, D // 2), u32),
            pltpu.VMEM((7 * (D // 4 + 64), D // 2), u32),
            pltpu.VMEM((7 * D // 4, D // 2), u32),
            pltpu.VMEM((NB * H // 2 * 64, T), u32),
            pltpu.VMEM((H // 2 * 64, T), u32),
            pltpu.VMEM((H // 2 * 32, T), u32),
            pltpu.VMEM((H // 2, 64, 128), f32),
            pltpu.VMEM((H // 2, 128, 128), f32),
            pltpu.VMEM((H // 2 * 40, 128), u32),
            pltpu.VMEM((7 * T // 4, D // 2), u32),
            pltpu.VMEM((NB, T, D), bf16),
            pltpu.SemaphoreType.DMA((NB,)),
            pltpu.SemaphoreType.DMA((12,)),
            pltpu.SemaphoreType.DMA((2,)),
            pltpu.SemaphoreType.DMA((NB,)),
            pltpu.SemaphoreType.DMA((4,)),
            pltpu.SemaphoreType.REGULAR,
        ],
        compiler_params=pltpu.CompilerParams(vmem_limit_bytes=120 * 1024 * 1024),
    )(x2, wqkv, w_phi, wo)
    return out.reshape(B, S, D)
```

```python
import numpy as np
import jax
import jax.numpy as jnp
from jax import lax
import jax.experimental.pallas as pl
import jax.experimental.pallas.tpu as pltpu

f32 = jnp.float32
bf16 = jnp.bfloat16
u32 = jnp.uint32
LOG2E = 1.4426950408889634
H = 32
DH = 32

_LHS = [[(1, 0, 0), (1, 1, 1)], [(1, 1, 0), (1, 1, 1)], [(1, 0, 0)], [(1, 1, 1)],
        [(1, 0, 0), (1, 0, 1)], [(1, 1, 0), (-1, 0, 0)], [(1, 0, 1), (-1, 1, 1)]]
_RHS = [[(1, 0, 0), (1, 1, 1)], [(1, 0, 0)], [(1, 0, 1), (-1, 1, 1)], [(1, 1, 0), (-1, 0, 0)],
        [(1, 1, 1)], [(1, 0, 0), (1, 0, 1)], [(1, 1, 0), (1, 1, 1)]]
_ORDER = [1, 4, 2, 3, 0, 6, 5]


def _nt(a, b):
    return lax.dot_general(a, b, (((1,), (1,)), ((), ())), preferred_element_type=f32)


def _nn(a, b):
    return jnp.dot(a, b, preferred_element_type=f32)


def _pk(x):
    return pltpu.bitcast(x.astype(bf16), u32)


def _up(x):
    return pltpu.bitcast(x, bf16)


def _rcp(s):
    r = pltpu.reciprocal(s, approx=True)
    return r * (2.0 - s * r)


def _allred(x, op):
    x = op(x, pltpu.roll(x, 4, 1))
    return op(x, pltpu.roll(x, 2, 1))


def _dual_softmax(p):
    R, Tn = p.shape
    p4 = p.reshape(R // 64, 8, 8, Tn)
    mx = _allred(jnp.max(p4, axis=1), jnp.maximum)[:, None]
    mn = _allred(jnp.min(p4, axis=1), jnp.minimum)[:, None]
    ep = jnp.exp2(p4 - mx)
    en = jnp.exp2(mn - p4)
    sp = _allred(jnp.sum(ep, axis=1), jnp.add)[:, None]
    sn = _allred(jnp.sum(en, axis=1), jnp.add)[:, None]
    pp = ep * _rcp(sp)
    pn = en * _rcp(sn)
    return jnp.concatenate([pp.reshape(R, Tn), pn.reshape(R, Tn)], axis=0)


def _combo(recipe, get):
    s, a, b = recipe[0]
    v = get(a, b)
    for s, a, b in recipe[1:]:
        v = v + get(a, b) if s > 0 else v - get(a, b)
    return v


def _two_level(table, n, get):
    cache = {}

    def g1(r2, c2):
        if (r2, c2) not in cache:
            cache[r2, c2] = _combo(table[n], lambda r1, c1: get(r1, c1, r2, c2))
        return cache[r2, c2]
    return [_combo(table[j], g1) for j in range(7)]


def _strassen(m, emit):
    m2 = m(1)
    m5 = m(4)
    m3 = m(2)
    t22 = _sub(m3, m2)
    emit(0, 1, _add(m3, m5))
    m4 = m(3)
    t11 = _sub(m4, m5)
    emit(1, 0, _add(m2, m4))
    m1 = m(0)
    t11 = _add(t11, m1)
    t22 = _add(t22, m1)
    m7 = m(6)
    emit(0, 0, _add(t11, m7))
    m6 = m(5)
    emit(1, 1, _add(t22, m6))


def _add(a, b):
    if isinstance(a, dict):
        return {k: a[k] + b[k] for k in a}
    return a + b


def _sub(a, b):
    if isinstance(a, dict):
        return {k: a[k] - b[k] for k in a}
    return a - b


def _strassen2(m, emit):
    def M(n):
        q = {}
        _strassen(lambda j: m(n, j), lambda a, b, v: q.__setitem__((a, b), v))
        return q

    def e1(a, b, q):
        for (c, d), v in q.items():
            emit(a, b, c, d, v)
    _strassen(M, e1)


class _Fill:
    def __init__(self, thunks):
        self.t = list(thunks)
        self.credit = 0.0

    def pop(self, n=1):
        self.credit += n
        while self.credit >= 1 and self.t:
            self.credit -= 1
            self.t.pop(0)()

    def drain(self):
        while self.t:
            self.t.pop(0)()


def make_kernel(S, D, T):
    NB = S // T
    NP = H // 2
    T2 = T // 2
    D2 = D // 2
    NG = 4
    Q = 256

    def kernel(x_hbm, wqkv_hbm, wphi_hbm, wo_hbm, o_hbm,
               stg, xu, wphi, abd, bufa, bufb, wtmp, phq, kvbd, ot, vo, ostage,
               xsem, gsem, wsem, osem, fsem, rsem):
        def mo(v, m):
            return v if isinstance(v, int) else pl.multiple_of(v, m)

        WO = S
        XB = 49 * 64
        KV = NB * XB
        VT = 3 * 49 * 128
        PH = 49 * 128

        def urow(u):
            return mo(S + D + D * (u // NG), D)

        def ucol(u):
            return mo(256 * (u % NG), 256)

        def x_copy(i):
            return pltpu.make_async_copy(x_hbm.at[pl.ds(i * T, T)], stg.at[pl.ds(i * T, T)], xsem.at[i])

        def u_copy(u):
            if isinstance(u, int):
                col = (D, 0, 2 * D)[u // NG] + 256 * (u % NG)
            else:
                blk = u // NG
                col = pl.multiple_of(jnp.where(blk == 0, D, jnp.where(blk == 1, 0, 2 * D)) + 256 * (u % NG), 256)
            return pltpu.make_async_copy(wqkv_hbm.at[:, pl.ds(col, 256)],
                                         stg.at[pl.ds(urow(u), D), pl.ds(ucol(u), 256)], gsem.at[u])

        phi_copy = pltpu.make_async_copy(wphi_hbm, wphi, wsem.at[0])
        wo_copy = pltpu.make_async_copy(wo_hbm, stg.at[pl.ds(WO, D)], wsem.at[1])

        phi_copy.start()
        pl.semaphore_signal(rsem, 1)
        pl.semaphore_wait(rsem, 1)
        u_copy(0).start()
        x_copy(0).start()
        u_copy(8).start()
        for g in range(1, NG):
            u_copy(g).start()
            u_copy(8 + g).start()
        for g in range(NG):
            u_copy(4 + g).start()
        x_copy(1).start()
        wo_copy.start()
        for i in range(2, NB):
            x_copy(i).start()

        def vview(s, r, nr):
            if isinstance(s, int) and s == 2:
                return bufb.at[pl.ds(mo(r, 32), 48 * 128 + nr)]
            if isinstance(s, int) and s == 3:
                s = 2
            return bufa.at[pl.ds(mo(49 * 128 * s + r, 32), 48 * 128 + nr)]

        def prep_thunks(table, s, g, get):
            dst = vview(s, 32 * g, 32)

            def one(rr, c):
                cache = {}

                def g_(*k):
                    if k not in cache:
                        cache[k] = get(*k, rr, c)
                    return cache[k]
                for n in [2, 4, 0, 6, 3, 1, 5]:
                    for j, op in enumerate(_two_level(table, n, g_)):
                        dst[pl.ds((7 * n + j) * 128 + 8 * rr, 8), 128 * c:128 * (c + 1)] = _pk(op)
            return [lambda rr=rr, c=c: one(rr, c) for c in range(2) for rr in range(4)]

        def wprep_mm(u):
            g = u % NG
            av = abd.at[pl.ds(mo(128 * g, 128), 128)]
            wv = stg.at[pl.ds(urow(u), D), pl.ds(ucol(u), 256)]

            def mm(c, hh):
                lhs = _up(av[pl.ds(64 * hh, 64), :])
                cs = pl.ds(128 * hh, 128)
                rhs = jnp.concatenate([wv[pl.ds(256 * qq + 128 * c, 128), cs] for qq in range(4)], axis=0)
                wt = _nt(lhs, rhs) * LOG2E
                for qq in range(4):
                    wtmp[64 * hh:64 * (hh + 1), 256 * qq + 128 * c:256 * qq + 128 * (c + 1)] = _pk(wt[:, 128 * qq:128 * (qq + 1)])
            return [lambda c=c, hh=hh: mm(c, hh) for c in range(2) for hh in range(2)]

        def wprep_st(u):
            def get(r1, c1, r2, c2, rr, c):
                r = 64 * r1 + 32 * r2 + 8 * rr
                d = 512 * c1 + 256 * c2 + 128 * c
                return _up(wtmp[r:r + 8, d:d + 128]).astype(f32)
            return prep_thunks(_LHS, u // NG, u % NG, get)

        def vprep_thunks(g):
            wv = stg.at[pl.ds(S + 3 * D, D), pl.ds(mo(256 * g, 256), 256)]

            def tr(hh, dt):
                w = wv[128 * dt:128 * (dt + 1), 128 * hh:128 * (hh + 1)].astype(f32).T
                wtmp[128 + 64 * hh:128 + 64 * (hh + 1), 128 * dt:128 * (dt + 1)] = _pk(w)

            def get(r1, c1, r2, c2, rr, c):
                r = 128 + 64 * r1 + 32 * r2 + 8 * rr
                d = 512 * c1 + 256 * c2 + 128 * c
                return _up(wtmp[r:r + 8, d:d + 128]).astype(f32)
            trs = [lambda hh=hh, dt=dt: tr(hh, dt) for dt in range(8) for hh in range(2)]
            return trs, prep_thunks(_LHS, 2, g, get)

        def xsum_thunks(xb, s0, by_op=False):
            src = stg.at[pl.ds(s0, T)]
            dst = xu.at[pl.ds(xb, XB)]

            def piece(rr, c, r1, c1, r2, c2):
                t = 256 * c1 + 128 * c2 + 16 * rr
                d = 512 * r1 + 256 * r2 + 128 * c
                return src[pl.ds(t, 16), d:d + 128].astype(f32)

            def put(n, rr, c, ops):
                for j, op in enumerate(ops):
                    dst[pl.ds((7 * n + j) * 64 + 8 * rr, 8), 128 * c:128 * (c + 1)] = _pk(op)

            def one_op(n, c):
                for rr in range(8):
                    put(n, rr, c, _two_level(_RHS, n, lambda *k: piece(rr, c, *k)))

            def one_chunk(rr, c):
                cache = {}

                def get(*k):
                    if k not in cache:
                        cache[k] = piece(rr, c, *k)
                    return cache[k]
                for n in [1, 5, 0, 2, 4, 6, 3]:
                    put(n, rr, c, _two_level(_RHS, n, get))
            if by_op:
                return [lambda n=n, c=c: one_op(n, c) for n in _ORDER for c in range(2)]
            return [lambda rr=rr, c=c: one_chunk(rr, c) for rr in range(8) for c in range(2)]

        def wosum_thunks(s):
            src, dst = stg.at[pl.ds(mo(WO + 64 * s, 64), D - 192)], vview(3, 32 * s, 32)

            def one(n, c):
                for rr in range(4):
                    def get(r1, c1, r2, c2):
                        r = 512 * r1 + 256 * r2 + 16 * rr
                        d = 512 * c1 + 256 * c2 + 128 * c
                        return src[pl.ds(r, 16), d:d + 128].astype(f32)
                    for j, op in enumerate(_two_level(_RHS, n, get)):
                        dst[pl.ds((7 * n + j) * 128 + 8 * rr, 8), 128 * c:128 * (c + 1)] = _pk(op)
            return [lambda n=n, c=c: one(n, c) for n in _ORDER for c in range(2)]

        def products(s, xb, g0, ng, emit, fill=None, per=0):
            lv, rv = vview(s, 32 * g0, 32 * ng), xu.at[pl.ds(mo(xb, 64), XB)]

            def m(n, j):
                lhs = _up(lv[pl.ds((7 * n + j) * 128, 32 * ng), :])
                rhs = _up(rv[pl.ds((7 * n + j) * 64, 64), :])
                r = _nt(lhs, rhs)
                if fill is not None:
                    fill.pop(per)
                return r

            def e(fh, th, f2, t2, c):
                for gg in range(ng):
                    emit(4 * gg + 2 * fh + f2, 2 * th + t2, c[64 * gg:64 * (gg + 1)])
            _strassen2(m, e)

        def k_emit(g0):
            dst = bufb.at[pl.ds(mo(PH + 256 * g0, 128), 1024 + (1024 if isinstance(g0, int) and g0 == 0 else 256))]

            def emit(p, tt, c):
                dst[pl.ds(1024 * (tt // 2) + 64 * p, 64), 128 * (tt % 2):128 * (tt % 2 + 1)] = _pk(_dual_softmax(c))
            return emit

        def v_emit(g0):
            dst = bufa.at[pl.ds(mo(VT + 160 * g0, 32), 640 + (640 if isinstance(g0, int) and g0 == 0 else 160))]

            def emit(p, tt, c):
                dst[pl.ds(640 * (tt // 2) + 40 * p, 32), 128 * (tt % 2):128 * (tt % 2 + 1)] = _pk(c)
            return emit

        def q_emit(i, g0, ng=1):
            dst = phq.at[pl.ds(mo(64 * NP * i + 256 * g0, 256), 256 * ng)]

            def emit(p, tt, c):
                dst[pl.ds(64 * p, 64), 128 * tt:128 * (tt + 1)] = _pk(_dual_softmax(c))
            return emit

        def kv_get(p):
            return pltpu.bitcast(xu[KV + 80 * p:KV + 80 * (p + 1), 0:128], f32)

        def kv_set(p, v):
            xu[KV + 80 * p:KV + 80 * (p + 1), 0:128] = pltpu.bitcast(v, u32)

        def kv_part(fill=None):
            for p in range(NP):
                lhs = jnp.concatenate([bufa[VT + 640 * th + 40 * p:VT + 640 * th + 40 * (p + 1), :] for th in range(2)], axis=1)
                rhs = jnp.concatenate([bufb[PH + 1024 * th + 64 * p:PH + 1024 * th + 64 * (p + 1), :] for th in range(2)], axis=1)
                kv_set(p, kv_get(p) + _nt(_up(lhs), _up(rhs)))
                if fill is not None:
                    fill.pop(1)

        def num_thunks(i, c):
            src = phq.at[pl.ds(mo(64 * NP * i, 64 * NP), 64 * NP)]

            def one(qq):
                halves = []
                for e in range(2):
                    p = 4 * qq + 2 * c + e
                    res = _nn(_up(kvbd[40 * p:40 * (p + 1), :]), _up(src[pl.ds(64 * p, 64), :]))
                    rd = _rcp(res[64:80] + 1e-6).reshape(2, 1, 8, T)
                    halves.append((res[0:64].reshape(2, 4, 8, T) * rd).reshape(64, T))
                oT = jnp.concatenate(halves, axis=0)
                ot[(4 * c + qq) * T:(4 * c + qq + 1) * T, :] = oT.T
            return [lambda qq=qq: one(qq) for qq in range(4)]

        def ov_thunk(c, n):
            def one():
                for rr in range(8):
                    def get(r1, c1, r2, c2):
                        r = (4 * c + 2 * c1 + c2) * T + 256 * r1 + 128 * r2 + 16 * rr
                        return ot[r:r + 16, :]
                    for j, op in enumerate(_two_level(_LHS, n, get)):
                        vo[(7 * n + j) * 64 + 8 * rr:(7 * n + j) * 64 + 8 * rr + 8, 128 * c:128 * (c + 1)] = _pk(op)
            return one

        def o_copy(i):
            return pltpu.make_async_copy(ostage.at[i], o_hbm.at[pl.ds(pl.multiple_of(i * T, T), T)], osem.at[i])

        def oq_copy(i, th, nh, t2=None, n2=None):
            if t2 is None:
                r, nr, c, nc, k = 256 * th, 256, 512 * nh, 512, 2 * th + nh
            else:
                r, nr, c, nc, k = 256 * th + 128 * t2, 128, 512 * nh + 256 * n2, 256, 4 + 2 * t2 + n2
            return pltpu.make_async_copy(ostage.at[i, pl.ds(r, nr), pl.ds(c, nc)],
                                         o_hbm.at[pl.ds(i * T + r, nr), pl.ds(c, nc)], fsem.at[k])

        def out_part(i, final, nxt=None):
            sched = {}
            if nxt is not None:
                n0, n1 = num_thunks(nxt, 0), num_thunks(nxt, 1)
                sched[0] = [n0[0], n0[1]]
                sched[2] = [n0[2]]
                sched[4] = [n0[3]]
                sched[6] = [n1[0]]
                sched[9] = [n1[1]]
                sched[12] = [n1[2]]
                sched[15] = [n1[3]]
                for k, n in enumerate(_ORDER):
                    done = 7 * (k + 1)
                    sched.setdefault(max(done + 1, 17), []).append(ov_thunk(0, n))
                    sched.setdefault(max(done + 3, 20), []).append(ov_thunk(1, n))
            cnt = [0]

            def side():
                for f in sched.pop(cnt[0], []):
                    f()

            side()

            def m(n, j):
                r = _nn(_up(vo[(7 * n + j) * 64:(7 * n + j + 1) * 64, :]), _up(bufa[(98 + 7 * n + j) * 128:(98 + 7 * n + j + 1) * 128, :]))
                cnt[0] += 1
                side()
                return r
            seen = {}

            def e(th, nh, t2, n2, c):
                r, col = 256 * th + 128 * t2, 512 * nh + 256 * n2
                ostage[i, r:r + 128, col:col + 256] = c.astype(bf16)
                if final:
                    seen[th, nh] = seen.get((th, nh), 0) + 1
                    if (th, nh) == (1, 1):
                        oq_copy(i, th, nh, t2, n2).start()
                    elif seen[th, nh] == 4:
                        oq_copy(i, th, nh).start()
            _strassen2(m, e)
            for k in sorted(sched):
                for f in sched[k]:
                    f()

        phi_copy.wait()
        r_s = lax.broadcasted_iota(jnp.int32, (128, DH), 0)
        c_s = lax.broadcasted_iota(jnp.int32, (128, DH), 1)
        sel = (((r_s % 64) // 2) == c_s).astype(f32).astype(bf16)
        r_m = lax.broadcasted_iota(jnp.int32, (128, 128), 0)
        c_m = lax.broadcasted_iota(jnp.int32, (128, 128), 1)
        hd_mask = (2 * (r_m // 64) + r_m % 2) == (c_m // DH)
        for gg in range(8):
            w4 = wphi[4 * gg:4 * gg + 4].reshape(128, DH)
            abd[64 * gg:64 * (gg + 1), :] = _pk(jnp.where(hd_mask, _nt(sel, w4), 0.0))
        for p in range(NP):
            kv_set(p, jnp.zeros((80, 128), f32))
            for th in range(2):
                bufa[VT + 640 * th + 40 * p + 32:VT + 640 * th + 40 * p + 40, :] = _pk(jnp.ones((16, T2), f32))
        u_copy(0).wait()
        _Fill(wprep_mm(0) + wprep_st(0)).drain()
        x_copy(0).wait()

        def group(g, first):
            trs, vst = vprep_thunks(g)
            if first:
                _Fill(xsum_thunks(0, 0, True)).drain()
                u_copy(8).wait()
            fill = _Fill(trs + vst)
            products(0, 0, g, 1, k_emit(g), fill, 24 / 45)
            fill.drain()
            if first:
                u_copy(1).wait()
            _Fill(wprep_mm(g + 1)).drain()
            fill = _Fill(wprep_st(g + 1))
            products(2, 0, g, 1, v_emit(g), fill, 8 / 40)
            fill.drain()

        group(0, True)

        def pbody(g, c):
            u_copy(8 + g).wait()
            u_copy(g + 1).wait()
            group(g, False)
            return c

        lax.fori_loop(1, NG, pbody, 0)
        for g in range(1, NG):
            u_copy(4 + g).wait()
        wo_copy.wait()
        fill = _Fill(wosum_thunks(0))
        for g in range(1, NG):
            _Fill(wprep_mm(4 + g) + wprep_st(4 + g)).drain()
            fill.pop(5)
        fill.drain()

        def kbody(i, c):
            x_copy(i).wait()
            s0 = pl.multiple_of(i * T, T)
            xb = pl.multiple_of(XB * (i - 1), 64)
            kv_part(_Fill(xsum_thunks(xb + XB, s0)))
            products(1, xb, 0, NG, q_emit(i - 1, 0, NG))
            products(0, xb + XB, 0, NG, k_emit(0))
            fw = _Fill(wosum_thunks(i))
            products(2, xb + XB, 0, NG, v_emit(0), fw, 14 / 45)
            fw.drain()
            return c

        lax.fori_loop(1, NB, kbody, 0)

        kv_part()
        products(1, XB * (NB - 1), 0, 1, q_emit(NB - 1, 0))
        r_k = lax.broadcasted_iota(jnp.int32, (80, 128), 0)
        m2_ = jnp.where(r_k < 64, r_k // 32, (r_k - 64) // 8) == (lax.broadcasted_iota(jnp.int32, (80, 128), 1) % 2)
        for p in range(NP):
            kvbd[40 * p:40 * (p + 1), :] = _pk(jnp.where(m2_, kv_get(p), 0.0))
        _Fill(num_thunks(0, 0)).drain()
        fill = _Fill([ov_thunk(0, n) for n in _ORDER[:3]])
        products(1, XB * (NB - 1), 1, 1, q_emit(NB - 1, 1), fill, 3 / 45)
        fill.drain()
        _Fill(num_thunks(0, 1)).drain()
        fill = _Fill([ov_thunk(0, n) for n in _ORDER[3:]] + [ov_thunk(1, n) for n in _ORDER[:3]])
        products(1, XB * (NB - 1), 2, 1, q_emit(NB - 1, 2), fill, 7 / 45)
        fill.drain()
        fill = _Fill([ov_thunk(1, n) for n in _ORDER[3:]])
        products(1, XB * (NB - 1), 3, 1, q_emit(NB - 1, 3), fill, 4 / 45)
        fill.drain()

        def qbody(i, c):
            out_part(i, False, i + 1)
            o_copy(i).start()
            return c

        lax.fori_loop(0, NB - 1, qbody, 0)

        out_part(NB - 1, True)
        for i in range(NB - 1):
            o_copy(i).wait()
        for th, nh in [(0, 1), (1, 0), (0, 0)]:
            oq_copy(NB - 1, th, nh).wait()
        for t2 in range(2):
            for n2 in range(2):
                oq_copy(NB - 1, 1, 1, t2, n2).wait()

    return kernel


@jax.jit
def pallas_standalone__linear_kernel_hedgehog__prompt_kernel(x, wqkv, w_phi, wo):
    B, S, D = x.shape
    T = 512
    x2 = x.reshape(S, D)
    NB = S // T
    out = pl.pallas_call(
        make_kernel(S, D, T),
        out_shape=jax.ShapeDtypeStruct((S, D), bf16),
        in_specs=[pl.BlockSpec(memory_space=pl.ANY)] * 4,
        out_specs=pl.BlockSpec(memory_space=pl.ANY),
        scratch_shapes=[
            pltpu.VMEM((S + 4 * D, D), bf16),
            pltpu.VMEM((NB * 49 * 64 + 1280, 256), u32),
            pltpu.VMEM((H, DH, DH), bf16),
            pltpu.VMEM((8 * 64, 128), u32),
            pltpu.VMEM((3 * 49 * 128 + 1280, 256), u32),
            pltpu.VMEM((49 * 128 + 2048, 256), u32),
            pltpu.VMEM((256, D), u32),
            pltpu.VMEM((NB * H // 2 * 64, T), u32),
            pltpu.VMEM((H // 2 * 40, 128), u32),
            pltpu.VMEM((8 * T, 128), f32),
            pltpu.VMEM((49 * 64, 256), u32),
            pltpu.VMEM((NB, T, D), bf16),
            pltpu.SemaphoreType.DMA((NB,)),
            pltpu.SemaphoreType.DMA((12,)),
            pltpu.SemaphoreType.DMA((2,)),
            pltpu.SemaphoreType.DMA((NB,)),
            pltpu.SemaphoreType.DMA((8,)),
            pltpu.SemaphoreType.REGULAR,
        ],
        compiler_params=pltpu.CompilerParams(vmem_limit_bytes=120 * 1024 * 1024),
    )(x2, wqkv, w_phi, wo)
    return out.reshape(B, S, D)
```

```python
import numpy as np
import jax
import jax.numpy as jnp
from jax import lax
import jax.experimental.pallas as pl
import jax.experimental.pallas.tpu as pltpu

f32 = jnp.float32
bf16 = jnp.bfloat16
u32 = jnp.uint32
LOG2E = 1.4426950408889634
H = 32
DH = 32

_LHS = [[(1, 0, 0), (1, 1, 1)], [(1, 1, 0), (1, 1, 1)], [(1, 0, 0)], [(1, 1, 1)],
        [(1, 0, 0), (1, 0, 1)], [(1, 1, 0), (-1, 0, 0)], [(1, 0, 1), (-1, 1, 1)]]
_RHS = [[(1, 0, 0), (1, 1, 1)], [(1, 0, 0)], [(1, 0, 1), (-1, 1, 1)], [(1, 1, 0), (-1, 0, 0)],
        [(1, 1, 1)], [(1, 0, 0), (1, 0, 1)], [(1, 1, 0), (1, 1, 1)]]
_ORDER = [1, 4, 2, 3, 0, 6, 5]


def _nt(a, b):
    return lax.dot_general(a, b, (((1,), (1,)), ((), ())), preferred_element_type=f32)


def _nn(a, b):
    return jnp.dot(a, b, preferred_element_type=f32)


def _pk(x):
    return pltpu.bitcast(x.astype(bf16), u32)


def _up(x):
    return pltpu.bitcast(x, bf16)


def _rcp(s):
    r = pltpu.reciprocal(s, approx=True)
    return r * (2.0 - s * r)


def _allred(x, op):
    x = op(x, pltpu.roll(x, 4, 1))
    return op(x, pltpu.roll(x, 2, 1))


def _dual_softmax(p):
    R, Tn = p.shape
    p4 = p.reshape(R // 64, 8, 8, Tn)
    mx = _allred(jnp.max(p4, axis=1), jnp.maximum)[:, None]
    mn = _allred(jnp.min(p4, axis=1), jnp.minimum)[:, None]
    ep = jnp.exp2(p4 - mx)
    en = jnp.exp2(mn - p4)
    sp = _allred(jnp.sum(ep, axis=1), jnp.add)[:, None]
    sn = _allred(jnp.sum(en, axis=1), jnp.add)[:, None]
    pp = ep * _rcp(sp)
    pn = en * _rcp(sn)
    return jnp.concatenate([pp.reshape(R, Tn), pn.reshape(R, Tn)], axis=0)


def _combo(recipe, get):
    s, a, b = recipe[0]
    v = get(a, b)
    for s, a, b in recipe[1:]:
        v = v + get(a, b) if s > 0 else v - get(a, b)
    return v


def _two_level(table, n, get):
    cache = {}

    def g1(r2, c2):
        if (r2, c2) not in cache:
            cache[r2, c2] = _combo(table[n], lambda r1, c1: get(r1, c1, r2, c2))
        return cache[r2, c2]
    return [_combo(table[j], g1) for j in range(7)]


def _strassen(m, emit):
    m2 = m(1)
    m5 = m(4)
    m3 = m(2)
    t22 = _sub(m3, m2)
    emit(0, 1, _add(m3, m5))
    m4 = m(3)
    t11 = _sub(m4, m5)
    emit(1, 0, _add(m2, m4))
    m1 = m(0)
    t11 = _add(t11, m1)
    t22 = _add(t22, m1)
    m7 = m(6)
    emit(0, 0, _add(t11, m7))
    m6 = m(5)
    emit(1, 1, _add(t22, m6))


def _add(a, b):
    if isinstance(a, dict):
        return {k: a[k] + b[k] for k in a}
    return a + b


def _sub(a, b):
    if isinstance(a, dict):
        return {k: a[k] - b[k] for k in a}
    return a - b


def _strassen2(m, emit):
    def M(n):
        q = {}
        _strassen(lambda j: m(n, j), lambda a, b, v: q.__setitem__((a, b), v))
        return q

    def e1(a, b, q):
        for (c, d), v in q.items():
            emit(a, b, c, d, v)
    _strassen(M, e1)


class _Fill:
    def __init__(self, thunks):
        self.t = list(thunks)
        self.credit = 0.0

    def pop(self, n=1):
        self.credit += n
        while self.credit >= 1 and self.t:
            self.credit -= 1
            self.t.pop(0)()

    def drain(self):
        while self.t:
            self.t.pop(0)()


def make_kernel(S, D, T):
    NB = S // T
    NP = H // 2
    T2 = T // 2
    D2 = D // 2
    NG = 4
    Q = 256

    def kernel(x_hbm, wqkv_hbm, wphi_hbm, wo_hbm, o_hbm,
               stg, xu, wphi, abd, bufa, bufb, wtmp, phq, kvbd, ot, vo, ostage,
               xsem, gsem, wsem, osem, fsem, rsem):
        def mo(v, m):
            return v if isinstance(v, int) else pl.multiple_of(v, m)

        WO = S
        XB = 49 * 64
        KV = NB * XB
        VT = 3 * 49 * 128
        PH = 49 * 128

        def urow(u):
            return mo(S + D + D * (u // NG), D)

        def ucol(u):
            return mo(256 * (u % NG), 256)

        def x_copy(i):
            return pltpu.make_async_copy(x_hbm.at[pl.ds(i * T, T)], stg.at[pl.ds(i * T, T)], xsem.at[i])

        def u_copy(u):
            if isinstance(u, int):
                col = (D, 0, 2 * D)[u // NG] + 256 * (u % NG)
            else:
                blk = u // NG
                col = pl.multiple_of(jnp.where(blk == 0, D, jnp.where(blk == 1, 0, 2 * D)) + 256 * (u % NG), 256)
            return pltpu.make_async_copy(wqkv_hbm.at[:, pl.ds(col, 256)],
                                         stg.at[pl.ds(urow(u), D), pl.ds(ucol(u), 256)], gsem.at[u])

        phi_copy = pltpu.make_async_copy(wphi_hbm, wphi, wsem.at[0])
        wo_copy = pltpu.make_async_copy(wo_hbm, stg.at[pl.ds(WO, D)], wsem.at[1])

        phi_copy.start()
        pl.semaphore_signal(rsem, 1)
        pl.semaphore_wait(rsem, 1)
        u_copy(0).start()
        x_copy(0).start()
        u_copy(8).start()
        for g in range(1, NG):
            u_copy(g).start()
            u_copy(8 + g).start()
        for g in range(NG):
            u_copy(4 + g).start()
        x_copy(1).start()
        wo_copy.start()
        for i in range(2, NB):
            x_copy(i).start()

        def vview(s, r, nr):
            if isinstance(s, int) and s == 2:
                return bufb.at[pl.ds(mo(r, 32), 48 * 128 + nr)]
            if isinstance(s, int) and s == 3:
                s = 2
            return bufa.at[pl.ds(mo(49 * 128 * s + r, 32), 48 * 128 + nr)]

        def prep_thunks(table, s, g, get):
            dst = vview(s, 32 * g, 32)

            def one(rr, c):
                cache = {}

                def g_(*k):
                    if k not in cache:
                        cache[k] = get(*k, rr, c)
                    return cache[k]
                for n in [2, 4, 0, 6, 3, 1, 5]:
                    for j, op in enumerate(_two_level(table, n, g_)):
                        dst[pl.ds((7 * n + j) * 128 + 8 * rr, 8), 128 * c:128 * (c + 1)] = _pk(op)
            return [lambda rr=rr, c=c: one(rr, c) for c in range(2) for rr in range(4)]

        def wprep_mm(u):
            g = u % NG
            av = abd.at[pl.ds(mo(128 * g, 128), 128)]
            wv = stg.at[pl.ds(urow(u), D), pl.ds(ucol(u), 256)]

            def mm(c, hh):
                lhs = _up(av[pl.ds(64 * hh, 64), :])
                cs = pl.ds(128 * hh, 128)
                rhs = jnp.concatenate([wv[pl.ds(256 * qq + 128 * c, 128), cs] for qq in range(4)], axis=0)
                wt = _nt(lhs, rhs) * LOG2E
                for qq in range(4):
                    wtmp[64 * hh:64 * (hh + 1), 256 * qq + 128 * c:256 * qq + 128 * (c + 1)] = _pk(wt[:, 128 * qq:128 * (qq + 1)])
            return [lambda c=c, hh=hh: mm(c, hh) for c in range(2) for hh in range(2)]

        def wprep_st(u):
            def get(r1, c1, r2, c2, rr, c):
                r = 64 * r1 + 32 * r2 + 8 * rr
                d = 512 * c1 + 256 * c2 + 128 * c
                return _up(wtmp[r:r + 8, d:d + 128]).astype(f32)
            return prep_thunks(_LHS, u // NG, u % NG, get)

        def vprep_thunks(g):
            wv = stg.at[pl.ds(S + 3 * D, D), pl.ds(mo(256 * g, 256), 256)]

            def tr(hh, dt):
                w = wv[128 * dt:128 * (dt + 1), 128 * hh:128 * (hh + 1)].astype(f32).T
                wtmp[128 + 64 * hh:128 + 64 * (hh + 1), 128 * dt:128 * (dt + 1)] = _pk(w)

            def get(r1, c1, r2, c2, rr, c):
                r = 128 + 64 * r1 + 32 * r2 + 8 * rr
                d = 512 * c1 + 256 * c2 + 128 * c
                return _up(wtmp[r:r + 8, d:d + 128]).astype(f32)
            trs = [lambda hh=hh, dt=dt: tr(hh, dt) for dt in range(8) for hh in range(2)]
            return trs, prep_thunks(_LHS, 2, g, get)

        def xsum_thunks(xb, s0, by_op=False):
            src = stg.at[pl.ds(s0, T)]
            dst = xu.at[pl.ds(xb, XB)]

            def piece(rr, c, r1, c1, r2, c2):
                t = 256 * c1 + 128 * c2 + 16 * rr
                d = 512 * r1 + 256 * r2 + 128 * c
                return src[pl.ds(t, 16), d:d + 128].astype(f32)

            def put(n, rr, c, ops):
                for j, op in enumerate(ops):
                    dst[pl.ds((7 * n + j) * 64 + 8 * rr, 8), 128 * c:128 * (c + 1)] = _pk(op)

            def one_op(n, c):
                for rr in range(8):
                    put(n, rr, c, _two_level(_RHS, n, lambda *k: piece(rr, c, *k)))

            def one_chunk(rr, c):
                cache = {}

                def get(*k):
                    if k not in cache:
                        cache[k] = piece(rr, c, *k)
                    return cache[k]
                for n in [1, 5, 0, 2, 4, 6, 3]:
                    put(n, rr, c, _two_level(_RHS, n, get))
            if by_op:
                return [lambda n=n, c=c: one_op(n, c) for n in _ORDER for c in range(2)]
            return [lambda rr=rr, c=c: one_chunk(rr, c) for rr in range(8) for c in range(2)]

        def wosum_thunks(s):
            src, dst = stg.at[pl.ds(mo(WO + 64 * s, 64), D - 192)], vview(3, 32 * s, 32)

            def one(rr, c):
                cache = {}

                def get(r1, c1, r2, c2):
                    k = (r1, c1, r2, c2)
                    if k not in cache:
                        r = 512 * r1 + 256 * r2 + 16 * rr
                        d = 512 * c1 + 256 * c2 + 128 * c
                        cache[k] = src[pl.ds(r, 16), d:d + 128].astype(f32)
                    return cache[k]
                for n in [1, 5, 0, 2, 4, 6, 3]:
                    for j, op in enumerate(_two_level(_RHS, n, get)):
                        dst[pl.ds((7 * n + j) * 128 + 8 * rr, 8), 128 * c:128 * (c + 1)] = _pk(op)
            return [lambda rr=rr, c=c: one(rr, c) for rr in range(4) for c in range(2)]

        def products(s, xb, g0, ng, emit, fill=None, per=0):
            lv, rv = vview(s, 32 * g0, 32 * ng), xu.at[pl.ds(mo(xb, 64), XB)]

            def m(n, j):
                lhs = _up(lv[pl.ds((7 * n + j) * 128, 32 * ng), :])
                rhs = _up(rv[pl.ds((7 * n + j) * 64, 64), :])
                r = _nt(lhs, rhs)
                if fill is not None:
                    fill.pop(per)
                return r

            def e(fh, th, f2, t2, c):
                for gg in range(ng):
                    emit(4 * gg + 2 * fh + f2, 2 * th + t2, c[64 * gg:64 * (gg + 1)])
            _strassen2(m, e)

        def k_emit(g0):
            dst = bufb.at[pl.ds(mo(PH + 256 * g0, 128), 1024 + (1024 if isinstance(g0, int) and g0 == 0 else 256))]

            def emit(p, tt, c):
                dst[pl.ds(1024 * (tt // 2) + 64 * p, 64), 128 * (tt % 2):128 * (tt % 2 + 1)] = _pk(_dual_softmax(c))
            return emit

        def v_emit(g0):
            dst = bufa.at[pl.ds(mo(VT + 160 * g0, 32), 640 + (640 if isinstance(g0, int) and g0 == 0 else 160))]

            def emit(p, tt, c):
                dst[pl.ds(640 * (tt // 2) + 40 * p, 32), 128 * (tt % 2):128 * (tt % 2 + 1)] = _pk(c)
            return emit

        def q_emit(i, g0, ng=1):
            dst = phq.at[pl.ds(mo(64 * NP * i + 256 * g0, 256), 256 * ng)]

            def emit(p, tt, c):
                dst[pl.ds(64 * p, 64), 128 * tt:128 * (tt + 1)] = _pk(_dual_softmax(c))
            return emit

        def kv_get(p):
            return pltpu.bitcast(xu[KV + 80 * p:KV + 80 * (p + 1), 0:128], f32)

        def kv_set(p, v):
            xu[KV + 80 * p:KV + 80 * (p + 1), 0:128] = pltpu.bitcast(v, u32)

        def kv_part(fill=None):
            for p in range(NP):
                lhs = jnp.concatenate([bufa[VT + 640 * th + 40 * p:VT + 640 * th + 40 * (p + 1), :] for th in range(2)], axis=1)
                rhs = jnp.concatenate([bufb[PH + 1024 * th + 64 * p:PH + 1024 * th + 64 * (p + 1), :] for th in range(2)], axis=1)
                kv_set(p, kv_get(p) + _nt(_up(lhs), _up(rhs)))
                if fill is not None:
                    fill.pop(1)

        def num_thunks(i, c):
            src = phq.at[pl.ds(mo(64 * NP * i, 64 * NP), 64 * NP)]

            def one(qq):
                halves = []
                for e in range(2):
                    p = 4 * qq + 2 * c + e
                    res = _nn(_up(kvbd[40 * p:40 * (p + 1), :]), _up(src[pl.ds(64 * p, 64), :]))
                    rd = _rcp(res[64:80] + 1e-6).reshape(2, 1, 8, T)
                    halves.append((res[0:64].reshape(2, 4, 8, T) * rd).reshape(64, T))
                oT = jnp.concatenate(halves, axis=0)
                ot[(4 * c + qq) * T:(4 * c + qq + 1) * T, :] = oT.T
            return [lambda qq=qq: one(qq) for qq in range(4)]

        def ov_thunk(c, n):
            def one():
                for rr in range(8):
                    def get(r1, c1, r2, c2):
                        r = (4 * c + 2 * c1 + c2) * T + 256 * r1 + 128 * r2 + 16 * rr
                        return ot[r:r + 16, :]
                    for j, op in enumerate(_two_level(_LHS, n, get)):
                        vo[(7 * n + j) * 64 + 8 * rr:(7 * n + j) * 64 + 8 * rr + 8, 128 * c:128 * (c + 1)] = _pk(op)
            return one

        def o_copy(i):
            return pltpu.make_async_copy(ostage.at[i], o_hbm.at[pl.ds(pl.multiple_of(i * T, T), T)], osem.at[i])

        def oq_copy(i, th, nh, t2=None, n2=None):
            if t2 is None:
                r, nr, c, nc, k = 256 * th, 256, 512 * nh, 512, 2 * th + nh
            else:
                r, nr, c, nc, k = 256 * th + 128 * t2, 128, 512 * nh + 256 * n2, 256, 4 + 2 * t2 + n2
            return pltpu.make_async_copy(ostage.at[i, pl.ds(r, nr), pl.ds(c, nc)],
                                         o_hbm.at[pl.ds(i * T + r, nr), pl.ds(c, nc)], fsem.at[k])

        def out_part(i, final, nxt=None):
            sched = {}
            if nxt is not None:
                n0, n1 = num_thunks(nxt, 0), num_thunks(nxt, 1)
                sched[0] = [n0[0], n0[1]]
                sched[2] = [n0[2]]
                sched[4] = [n0[3]]
                sched[6] = [n1[0]]
                sched[9] = [n1[1]]
                sched[12] = [n1[2]]
                sched[15] = [n1[3]]
                for k, n in enumerate(_ORDER):
                    done = 7 * (k + 1)
                    sched.setdefault(max(done + 1, 17), []).append(ov_thunk(0, n))
                    sched.setdefault(max(done + 3, 20), []).append(ov_thunk(1, n))
            cnt = [0]

            def side():
                for f in sched.pop(cnt[0], []):
                    f()

            side()

            def m(n, j):
                r = _nn(_up(vo[(7 * n + j) * 64:(7 * n + j + 1) * 64, :]), _up(bufa[(98 + 7 * n + j) * 128:(98 + 7 * n + j + 1) * 128, :]))
                cnt[0] += 1
                side()
                return r
            seen = {}

            def e(th, nh, t2, n2, c):
                r, col = 256 * th + 128 * t2, 512 * nh + 256 * n2
                ostage[i, r:r + 128, col:col + 256] = c.astype(bf16)
                if final:
                    seen[th, nh] = seen.get((th, nh), 0) + 1
                    if (th, nh) == (1, 1):
                        oq_copy(i, th, nh, t2, n2).start()
                    elif seen[th, nh] == 4:
                        oq_copy(i, th, nh).start()
            _strassen2(m, e)
            for k in sorted(sched):
                for f in sched[k]:
                    f()

        phi_copy.wait()
        r_s = lax.broadcasted_iota(jnp.int32, (128, DH), 0)
        c_s = lax.broadcasted_iota(jnp.int32, (128, DH), 1)
        sel = (((r_s % 64) // 2) == c_s).astype(f32).astype(bf16)
        r_m = lax.broadcasted_iota(jnp.int32, (128, 128), 0)
        c_m = lax.broadcasted_iota(jnp.int32, (128, 128), 1)
        hd_mask = (2 * (r_m // 64) + r_m % 2) == (c_m // DH)
        for gg in range(8):
            w4 = wphi[4 * gg:4 * gg + 4].reshape(128, DH)
            abd[64 * gg:64 * (gg + 1), :] = _pk(jnp.where(hd_mask, _nt(sel, w4), 0.0))
        for p in range(NP):
            kv_set(p, jnp.zeros((80, 128), f32))
            for th in range(2):
                bufa[VT + 640 * th + 40 * p + 32:VT + 640 * th + 40 * p + 40, :] = _pk(jnp.ones((16, T2), f32))
        u_copy(0).wait()
        _Fill(wprep_mm(0) + wprep_st(0)).drain()
        x_copy(0).wait()

        def group(g, first):
            trs, vst = vprep_thunks(g)
            if first:
                _Fill(xsum_thunks(0, 0, True)).drain()
                u_copy(8).wait()
            fill = _Fill(trs + vst)
            products(0, 0, g, 1, k_emit(g), fill, 24 / 45)
            fill.drain()
            if first:
                u_copy(1).wait()
            _Fill(wprep_mm(g + 1)).drain()
            fill = _Fill(wprep_st(g + 1))
            products(2, 0, g, 1, v_emit(g), fill, 8 / 40)
            fill.drain()

        group(0, True)

        def pbody(g, c):
            u_copy(8 + g).wait()
            u_copy(g + 1).wait()
            group(g, False)
            return c

        lax.fori_loop(1, NG, pbody, 0)
        for g in range(1, NG):
            u_copy(4 + g).wait()
        wo_copy.wait()
        fill = _Fill(wosum_thunks(0))
        for g in range(1, NG):
            _Fill(wprep_mm(4 + g) + wprep_st(4 + g)).drain()
            fill.pop(3)
        fill.drain()

        def kbody(i, c):
            x_copy(i).wait()
            s0 = pl.multiple_of(i * T, T)
            xb = pl.multiple_of(XB * (i - 1), 64)
            kv_part(_Fill(xsum_thunks(xb + XB, s0)))
            fw = _Fill(wosum_thunks(i))
            products(1, xb, 0, NG, q_emit(i - 1, 0, NG), fw, 8 / 18)
            products(0, xb + XB, 0, NG, k_emit(0))
            products(2, xb + XB, 0, NG, v_emit(0))
            return c

        lax.fori_loop(1, NB, kbody, 0)

        kv_part()
        products(1, XB * (NB - 1), 0, 1, q_emit(NB - 1, 0))
        r_k = lax.broadcasted_iota(jnp.int32, (80, 128), 0)
        m2_ = jnp.where(r_k < 64, r_k // 32, (r_k - 64) // 8) == (lax.broadcasted_iota(jnp.int32, (80, 128), 1) % 2)
        for p in range(NP):
            kvbd[40 * p:40 * (p + 1), :] = _pk(jnp.where(m2_, kv_get(p), 0.0))
        _Fill(num_thunks(0, 0)).drain()
        fill = _Fill([ov_thunk(0, n) for n in _ORDER[:3]])
        products(1, XB * (NB - 1), 1, 1, q_emit(NB - 1, 1), fill, 3 / 45)
        fill.drain()
        _Fill(num_thunks(0, 1)).drain()
        fill = _Fill([ov_thunk(0, n) for n in _ORDER[3:]] + [ov_thunk(1, n) for n in _ORDER[:3]])
        products(1, XB * (NB - 1), 2, 1, q_emit(NB - 1, 2), fill, 7 / 45)
        fill.drain()
        fill = _Fill([ov_thunk(1, n) for n in _ORDER[3:]])
        products(1, XB * (NB - 1), 3, 1, q_emit(NB - 1, 3), fill, 4 / 45)
        fill.drain()

        def qbody(i, c):
            out_part(i, False, i + 1)
            o_copy(i).start()
            return c

        lax.fori_loop(0, NB - 1, qbody, 0)

        out_part(NB - 1, True)
        for i in range(NB - 1):
            o_copy(i).wait()
        for th, nh in [(0, 1), (1, 0), (0, 0)]:
            oq_copy(NB - 1, th, nh).wait()
        for t2 in range(2):
            for n2 in range(2):
                oq_copy(NB - 1, 1, 1, t2, n2).wait()

    return kernel


@jax.jit
def pallas_standalone__linear_kernel_hedgehog__prompt_kernel(x, wqkv, w_phi, wo):
    B, S, D = x.shape
    T = 512
    x2 = x.reshape(S, D)
    NB = S // T
    out = pl.pallas_call(
        make_kernel(S, D, T),
        out_shape=jax.ShapeDtypeStruct((S, D), bf16),
        in_specs=[pl.BlockSpec(memory_space=pl.ANY)] * 4,
        out_specs=pl.BlockSpec(memory_space=pl.ANY),
        scratch_shapes=[
            pltpu.VMEM((S + 4 * D, D), bf16),
            pltpu.VMEM((NB * 49 * 64 + 1280, 256), u32),
            pltpu.VMEM((H, DH, DH), bf16),
            pltpu.VMEM((8 * 64, 128), u32),
            pltpu.VMEM((3 * 49 * 128 + 1280, 256), u32),
            pltpu.VMEM((49 * 128 + 2048, 256), u32),
            pltpu.VMEM((256, D), u32),
            pltpu.VMEM((NB * H // 2 * 64, T), u32),
            pltpu.VMEM((H // 2 * 40, 128), u32),
            pltpu.VMEM((8 * T, 128), f32),
            pltpu.VMEM((49 * 64, 256), u32),
            pltpu.VMEM((NB, T, D), bf16),
            pltpu.SemaphoreType.DMA((NB,)),
            pltpu.SemaphoreType.DMA((12,)),
            pltpu.SemaphoreType.DMA((2,)),
            pltpu.SemaphoreType.DMA((NB,)),
            pltpu.SemaphoreType.DMA((8,)),
            pltpu.SemaphoreType.REGULAR,
        ],
        compiler_params=pltpu.CompilerParams(vmem_limit_bytes=120 * 1024 * 1024),
    )(x2, wqkv, w_phi, wo)
    return out.reshape(B, S, D)
```
